```python
import os as _os
_os.environ.setdefault("JAX_PLATFORMS", "cpu")
import jax
import jax.numpy as jnp

def _softmax(x, axis=-1):
    return jax.nn.softmax(x, axis=axis)
def _gelu(x):
    return jax.nn.gelu(x, approximate=True)
def _silu(x):
    return jax.nn.silu(x)
def _sigmoid(x):
    return jax.nn.sigmoid(x)
def _layernorm(x, axis=-1, eps=1e-5):
    m = jnp.mean(x, axis=axis, keepdims=True)
    v = jnp.var(x, axis=axis, keepdims=True)
    return (x - m) / jnp.sqrt(v + eps)
def _scatter_add(tgt, idx, src, axis=0):
    return tgt.at[idx].add(src)
def _segment_sum(src, seg, n):
    return jax.ops.segment_sum(src, seg, n)
class _Rng:
    def __init__(self, key):
        self._k = key
    def _next(self):
        self._k, sub = jax.random.split(self._k)
        return sub
    def normal(self, shape):
        return jax.random.normal(self._next(), shape, dtype=jnp.bfloat16)
    def randint(self, lo, hi, shape):
        return jax.random.randint(self._next(), shape, lo, hi, dtype=jnp.int32)
    def uniform(self, shape, lo=0.0, hi=1.0):
        return jax.random.uniform(self._next(), shape, jnp.bfloat16, lo, hi)
    def permutation(self, n):
        return jax.random.permutation(self._next(), n)


kernel_name = 'parallel_sum__sliding_local_dilated__geglu_ffn__prompt'

def setup_inputs():
    _rng = _Rng(jax.random.key(int.from_bytes(__import__("os").urandom(4), "little")))
    _w = (lambda a: (lambda t: t.astype(jnp.bfloat16) if jnp.issubdtype(t.dtype, jnp.floating) else t)(jnp.asarray(a)))
    def _A_setup():
        B, S, D = 1, 2048, 640
        return {
            "x": _w((lambda *s: _rng.normal(s) * 0.05)(B, S, D)),
            "wqkv": _w((lambda *s: _rng.normal(s) * 0.05)(D, 3 * D)),
            "wo": _w((lambda *s: _rng.normal(s) * 0.05)(D, D)),
        }
    _A_in = _A_setup()

    def _B_setup():
        B, S, D, F = 1, 2048, 640, 1728
        return {
            "x": _w((lambda *s: _rng.normal(s) * 0.05)(B, S, D)),
            "w_gate": _w((lambda *s: _rng.normal(s) * 0.05)(D, F)),
            "w_up": _w((lambda *s: _rng.normal(s) * 0.05)(D, F)),
            "w_down": _w((lambda *s: _rng.normal(s) * 0.05)(F, D)),
        }
    _B_in = _B_setup()

    return {
        "A_x": _A_in["x"],
        "A_wqkv": _A_in["wqkv"],
        "A_wo": _A_in["wo"],
        "B_x": _B_in["x"],
        "B_w_gate": _B_in["w_gate"],
        "B_w_up": _B_in["w_up"],
        "B_w_down": _B_in["w_down"],
    }

def reference(A_x, A_wqkv, A_wo, B_x, B_w_gate, B_w_up, B_w_down):
    def _A_ref(x, wqkv, wo):
        B, S, D = x.shape
        H = 32; Dh = D // H
        W, dil = 8, 2
        qkv = (lambda x, *d: x.transpose(*d))((x @ wqkv).reshape(B, S, 3, H, Dh), 2, 0, 3, 1, 4)
        q, k, v = qkv[0], qkv[1], qkv[2]
        scale = Dh ** -0.5
        pos = jnp.arange(S)
        off = jnp.arange(W) * dil
        idx = pos[:, None] - off[None, :]
        mask = idx >= 0
        idx_c = jnp.where(mask, idx, 0).reshape(-1)
        kg = k[:, :, idx_c, :].reshape(B, H, S, W, Dh)
        vg = v[:, :, idx_c, :].reshape(B, H, S, W, Dh)
        logits = jnp.einsum("bhsd,bhswd->bhsw", q, kg) * scale
        logits = jnp.where(mask[None, None, :, :], logits, -1e9)
        attn = _softmax(logits, axis=-1)
        o = jnp.einsum("bhsw,bhswd->bhsd", attn, vg)
        return (lambda x, *d: x.transpose(*d))(o, 0, 2, 1, 3).reshape(B, S, D) @ wo

    def _B_ref(x, w_gate, w_up, w_down):
        return (_gelu(x @ w_gate) * (x @ w_up)) @ w_down

    x = A_x
    xn = _layernorm(x, axis=-1)
    return x + _A_ref(xn, A_wqkv, A_wo) + _B_ref(xn, B_w_gate, B_w_up, B_w_down)
```

```python
import functools
import jax
import jax.numpy as jnp
from jax import lax
import jax.experimental.pallas as pl
import jax.experimental.pallas.tpu as pltpu

S, D, F = 2048, 640, 1728
H, DH, W, DIL = 32, 20, 8, 2
T = 256
NT = S // T
HALO = 16
NC = D // 128
LOG2E = 1.4426950408889634
RC = 8
CHAIN = 2
CHAIN0 = 4
FM = 1664
NT_DIMS = (((1,), (1,)), ((), ()))
GU_CHUNKS = [(0, 256), (256, 640), (640, 1152), (1152, 1664)]
WD_CHUNKS = [(0, 896), (896, 1728)]
f32 = jnp.float32
bf16 = jnp.bfloat16


def _gelu(x):
    c = 0.7978845608028654
    inner = x * (c + (c * 0.044715) * (x * x))
    return (0.5 * x) * (1.0 + jnp.tanh(inner))


def _ln(x):
    x = x.astype(f32)
    m = jnp.mean(x, axis=-1, keepdims=True)
    xc = x - m
    var = jnp.mean(xc * xc, axis=-1, keepdims=True)
    return (xc * lax.rsqrt(var + 1e-5)).astype(bf16)


def _perm_cols(src_ref, dst_ref, p):
    R = D // 2
    lane = lax.broadcasted_iota(jnp.int32, (R, 128), 1)
    w = [pltpu.bitcast(src_ref[:, p * D + i * 128: p * D + (i + 1) * 128], jnp.uint32) for i in range(NC)]
    for j in range(NC):
        rel = (lane + (128 - 4 * j)) % 128
        h = (13 * (rel // 4)) % 32
        c = 20 * h + 4 * j + (rel % 4)
        s = w[4]
        for i in (3, 2, 1, 0):
            s = jnp.where(c < 128 * (i + 1), w[i], s)
        idx = (20 * (lane % 32) + 4 * j + lane // 32) % 128
        g = jnp.take_along_axis(s, idx, axis=1)
        dst_ref[:, p * D + j * 128: p * D + (j + 1) * 128] = pltpu.bitcast(g, bf16)


def _perm_rows(src_ref, tmp_ref, dst_ref):
    for j in range(NC):
        tmp_ref[j] = src_ref[:, j * 128:(j + 1) * 128].astype(f32)
    for d in range(DH):
        for j in range(NC):
            dst_ref[d * H:(d + 1) * H, j * 128:(j + 1) * 128] = (
                tmp_ref[j, pl.ds(d, H, stride=DH), :].astype(bf16))


def _attention(q_s, k_s, v_s, a_s, last, first, chain):
    qs = (DH ** -0.5) * LOG2E
    dens = []
    for c in range(T // RC):
        r0 = c * RC
        if c >= chain:
            sc = qs + jnp.minimum(dens[c - chain], 0.0)
        else:
            sc = qs + jnp.minimum(jnp.abs(last), 0.0)
        q = [q_s[j, r0:r0 + RC, :] * sc for j in range(NC)]
        ls = []
        for w in range(W):
            off = HALO + r0 - DIL * w
            p = q[0] * k_s[0, off:off + RC, :]
            for j in range(1, NC):
                p = p + q[j] * k_s[j, off:off + RC, :]
            p = p + pltpu.roll(p, 64, 1)
            p = p + pltpu.roll(p, 32, 1)
            if first and r0 < DIL * w:
                rows = r0 + lax.broadcasted_iota(jnp.int32, (RC, 128), 0)
                p = jnp.where(rows >= DIL * w, p, -1e9)
            ls.append(p)
        mx = jnp.maximum(jnp.maximum(jnp.maximum(ls[0], ls[1]), jnp.maximum(ls[2], ls[3])),
                         jnp.maximum(jnp.maximum(ls[4], ls[5]), jnp.maximum(ls[6], ls[7])))
        es = [jnp.exp2(l - mx) for l in ls]
        den = ((es[0] + es[1]) + (es[2] + es[3])) + ((es[4] + es[5]) + (es[6] + es[7]))
        dens.append(den)
        inv = pl.reciprocal(den, approx=False)
        for j in range(NC):
            acc = None
            for w in range(W):
                off = HALO + r0 - DIL * w
                t = es[w] * v_s[j, off:off + RC, :]
                acc = t if acc is None else acc + t
            a_s[r0:r0 + RC, j * 128:(j + 1) * 128] = (acc * inv).astype(bf16)


def kernel(x_hbm, wqkv_hbm, wo_hbm, wg_hbm, wu_hbm, wd_hbm, o_hbm,
           x_v, o_v, wqkv_raw, wqkv_p, wo_raw, wo_tmp, wo_p, wg_v, wu_v, wl_v, wd_v,
           xn_s, q_s, k_s, v_s, a_s, sem_x, sem_o, sem_w):
    def x_copy(i):
        return pltpu.make_async_copy(x_hbm.at[pl.ds(i * T, T)], x_v.at[pl.ds(i * T, T)], sem_x.at[i])

    def o_copy(i):
        return pltpu.make_async_copy(o_v.at[pl.ds(i * T, T)], o_hbm.at[pl.ds(i * T, T)], sem_o.at[i])

    n = [0]
    def wcopy(src, dst):
        c = pltpu.make_async_copy(src, dst, sem_w.at[n[0]])
        n[0] += 1
        return c

    gu_cp = [(wcopy(wg_hbm.at[a:b], wg_v.at[a:b]), wcopy(wu_hbm.at[a:b], wu_v.at[a:b])) for a, b in GU_CHUNKS]
    wl_cp = (wcopy(wg_hbm.at[FM:F], wl_v.at[0:64]), wcopy(wu_hbm.at[FM:F], wl_v.at[64:128]))
    qkv_cp = [wcopy(wqkv_hbm.at[:, p * D:(p + 1) * D], wqkv_raw.at[:, p * D:(p + 1) * D]) for p in range(3)]
    wd_cp = [wcopy(wd_hbm.at[a:b], wd_v.at[a:b]) for a, b in WD_CHUNKS]
    wo_cp = wcopy(wo_hbm, wo_raw)

    x_copy(0).start()
    for c in wl_cp:
        c.start()
    for cg, cu in gu_cp:
        cg.start()
        cu.start()
    for c in qkv_cp:
        c.start()
    for c in wd_cp:
        c.start()
    wo_cp.start()
    for i in range(1, NT):
        x_copy(i).start()

    k_s[:, 0:HALO, :] = jnp.zeros((NC, HALO, 128), f32)
    v_s[:, 0:HALO, :] = jnp.zeros((NC, HALO, 128), f32)

    x_copy(0).wait()
    xn = _ln(x_v[0:T, :])
    for c in wl_cp:
        c.wait()
    hs = []
    for ci, (a, b) in enumerate(GU_CHUNKS):
        gu_cp[ci][0].wait()
        gu_cp[ci][1].wait()
        if ci == 0:
            gu = lax.dot_general(xn, wl_v[...], NT_DIMS, preferred_element_type=f32)
            hl = (_gelu(gu) * pltpu.roll(gu, 64, 1))[:, 0:64].astype(bf16)
        if ci == len(GU_CHUNKS) - 1:
            qkv_cp[0].wait()
            _perm_cols(wqkv_raw, wqkv_p, 0)
        g = lax.dot_general(xn, wg_v[a:b, :], NT_DIMS, preferred_element_type=f32)
        u = lax.dot_general(xn, wu_v[a:b, :], NT_DIMS, preferred_element_type=f32)
        hs.append((_gelu(g) * u).astype(bf16))
    h = jnp.concatenate(hs + [hl], axis=1)
    for p, dst in enumerate((q_s, k_s, v_s)):
        if p < 2:
            qkv_cp[p + 1].wait()
            _perm_cols(wqkv_raw, wqkv_p, p + 1)
        else:
            wd_cp[0].wait()
        r = jnp.dot(xn, wqkv_p[:, p * D:(p + 1) * D], preferred_element_type=f32)
        o = 0 if p == 0 else HALO
        for j in range(NC):
            dst[j, o:o + T, :] = r[:, j * 128:(j + 1) * 128]
    last = r[T - RC:T, D - 128:D]
    a0, b0 = WD_CHUNKS[0]
    y = jnp.dot(h[:, a0:b0], wd_v[a0:b0, :], preferred_element_type=f32)
    wd_cp[1].wait()
    wo_cp.wait()
    x_copy(1).wait()
    _perm_rows(wo_raw, wo_tmp, wo_p)
    _attention(q_s, k_s, v_s, a_s, last, True, CHAIN0)
    a1, b1 = WD_CHUNKS[1]
    y = y + jnp.dot(h[:, a1:b1], wd_v[a1:b1, :], preferred_element_type=f32)
    y = y + jnp.dot(a_s[...], wo_p[...], preferred_element_type=f32)
    o_v[0:T, :] = (x_v[0:T, :].astype(f32) + y).astype(bf16)
    xn_s[...] = _ln(x_v[T:2 * T, :])
    o_copy(0).start()

    def body(i, carry):
        r_cur = pl.multiple_of(i * T, T)
        inext = jnp.minimum(i + 1, NT - 1)
        r_next = pl.multiple_of(inext * T, T)

        @pl.when(i + 1 < NT)
        def _():
            x_copy(inext).wait()

        k_s[:, 0:HALO, :] = k_s[:, T:T + HALO, :]
        v_s[:, 0:HALO, :] = v_s[:, T:T + HALO, :]
        xn = xn_s[...]
        xn_next = _ln(x_v[pl.ds(r_next, T), :])
        gu = lax.dot_general(xn, wl_v[...], NT_DIMS, preferred_element_type=f32)
        hl = (_gelu(gu) * pltpu.roll(gu, 64, 1))[:, 0:64].astype(bf16)
        qkv = jnp.dot(xn, wqkv_p[...], preferred_element_type=f32)
        for j in range(NC):
            q_s[j] = qkv[:, j * 128:(j + 1) * 128]
            k_s[j, HALO:HALO + T, :] = qkv[:, D + j * 128:D + (j + 1) * 128]
            v_s[j, HALO:HALO + T, :] = qkv[:, 2 * D + j * 128:2 * D + (j + 1) * 128]
        last = qkv[T - RC:T, 3 * D - 128:3 * D]
        _attention(q_s, k_s, v_s, a_s, last, False, CHAIN)
        g = lax.dot_general(xn, wg_v[...], NT_DIMS, preferred_element_type=f32)
        u = lax.dot_general(xn, wu_v[...], NT_DIMS, preferred_element_type=f32)
        h = (_gelu(g) * u).astype(bf16)
        y = jnp.dot(h, wd_v[0:FM, :], preferred_element_type=f32)
        y = y + jnp.dot(hl, wd_v[FM:F, :], preferred_element_type=f32)
        y = y + jnp.dot(a_s[...], wo_p[...], preferred_element_type=f32)
        o_v[pl.ds(r_cur, T), :] = (x_v[pl.ds(r_cur, T), :].astype(f32) + y).astype(bf16)
        xn_s[...] = xn_next
        o_copy(i).start()
        return carry

    lax.fori_loop(1, NT, body, 0)
    for i in range(NT):
        o_copy(i).wait()


@jax.jit
def pallas_parallel_sum__sliding_local_dilated__geglu_ffn__prompt_kernel(
    A_x, A_wqkv, A_wo, B_x, B_w_gate, B_w_up, B_w_down):
    x = A_x.reshape(S, D)
    anyspec = pl.BlockSpec(memory_space=pl.ANY)
    nw = 2 * len(GU_CHUNKS) + 2 + 3 + len(WD_CHUNKS) + 1
    out = pl.pallas_call(
        kernel,
        in_specs=[anyspec] * 6,
        out_specs=anyspec,
        out_shape=jax.ShapeDtypeStruct((S, D), bf16),
        scratch_shapes=[pltpu.VMEM((S, D), bf16),
                        pltpu.VMEM((S, D), bf16),
                        pltpu.VMEM((D, 3 * D), bf16),
                        pltpu.VMEM((D, 3 * D), bf16),
                        pltpu.VMEM((D, D), bf16),
                        pltpu.VMEM((NC, D, 128), f32),
                        pltpu.VMEM((D, D), bf16),
                        pltpu.VMEM((FM, D), bf16),
                        pltpu.VMEM((FM, D), bf16),
                        pltpu.VMEM((128, D), bf16),
                        pltpu.VMEM((F, D), bf16),
                        pltpu.VMEM((T, D), bf16),
                        pltpu.VMEM((NC, T, 128), f32),
                        pltpu.VMEM((NC, T + HALO, 128), f32),
                        pltpu.VMEM((NC, T + HALO, 128), f32),
                        pltpu.VMEM((T, D), bf16),
                        pltpu.SemaphoreType.DMA((NT,)),
                        pltpu.SemaphoreType.DMA((NT,)),
                        pltpu.SemaphoreType.DMA((nw,))],
        compiler_params=pltpu.CompilerParams(vmem_limit_bytes=100 * 1024 * 1024),
    )(x, A_wqkv, A_wo, B_w_gate.T, B_w_up.T, B_w_down)
    return out.reshape(1, S, D)
```

```python
import functools
import jax
import jax.numpy as jnp
from jax import lax
import jax.experimental.pallas as pl
import jax.experimental.pallas.tpu as pltpu

S, D, F = 2048, 640, 1728
H, DH, W, DIL = 32, 20, 8, 2
T0 = 528
T = 304
NL = (S - T0) // T
assert T0 + NL * T == S
TM = max(T0, T)
XPIECES = [(0, 144), (144, 272), (272, 400), (400, 528)]
HALO = 16
NC = D // 128
LOG2E = 1.4426950408889634
RC = 16
CHAIN = 1
CHAIN0 = 1
LN_IN_CHAIN = True
RA = 16
ROLL3 = False
RECIP = 1
LINK = 0
TRIG = True
ATT_T0 = 19.9
ATT_DT = 1.0
P_T0 = 11.9
P_DT = 0.62
PLN_T0 = 5.0
PLN_DT = 0.3
MID = 256
LN_T0 = 3.0
LN_DT = 0.8
LN_TRIG = True
FM = 1664
NT_DIMS = (((1,), (1,)), ((), ()))
GU_CHUNKS = [(0, 256), (256, 768), (768, 1152), (1152, 1664)]
f32 = jnp.float32
bf16 = jnp.bfloat16
u32 = jnp.uint32


def _pk(x):
    return pltpu.bitcast(x, u32)


def _upk(x):
    return pltpu.bitcast(x, bf16)


def _gelu(x):
    c = 0.7978845608028654
    inner = x * (c + (c * 0.044715) * (x * x))
    return (0.5 * x) * (1.0 + jnp.tanh(inner))


def _ln(x, z=None):
    x = x.astype(f32)
    if z is None:
        m = jnp.mean(x, axis=-1, keepdims=True)
    else:
        t = z + x[:, 0:128]
        for j in range(1, NC):
            t = t + x[:, j * 128:(j + 1) * 128]
        m = jnp.sum(t, axis=-1, keepdims=True) * (1.0 / D)
    xc = x - m
    var = jnp.mean(xc * xc, axis=-1, keepdims=True)
    rstd = lax.rsqrt(var + 1e-5)
    return (xc * rstd).astype(bf16), rstd


def _perm_cols(src_ref, dst_ref, p):
    R = D // 2
    lane = lax.broadcasted_iota(jnp.int32, (8, 128), 1)
    outs = []
    for j in range(NC):
        rel = (lane + (128 - 4 * j)) & 127
        h = (13 * (rel >> 2)) & 31
        c = jnp.tile(20 * h + 4 * j + (rel & 3), (R // 8, 1))
        idx = jnp.tile((20 * (lane & 31) + 4 * j + (lane >> 5)) & 127, (R // 8, 1))
        w = [_pk(src_ref[:, p * D + i * 128: p * D + (i + 1) * 128]) for i in range(NC)]
        s = w[4]
        for i in (3, 2, 1, 0):
            s = jnp.where(c < 128 * (i + 1), w[i], s)
        g = jnp.take_along_axis(s, idx, axis=1)
        dst_ref[:, p * D + j * 128: p * D + (j + 1) * 128] = g
        outs.append(_upk(g))
    return jnp.concatenate(outs, axis=1)


def _perm_rows(tmp_refs, dst_ref, z):
    cols = []
    for j in range(NC):
        blk = jnp.concatenate(
            [tmp_refs[j][z, pl.ds(d, H, stride=DH), :].astype(bf16) for d in range(DH)], axis=0)
        dst_ref[:, j * 128:(j + 1) * 128] = _pk(blk)
        cols.append(blk)
    return jnp.concatenate(cols, axis=1)


def _pick(tiles, rows, t):
    best = None
    for rnd, val in tiles:
        if rnd + 1 <= t:
            continue
        frac = max(t - rnd, 0.0)
        ro = min(8 * int(frac * rows / 8), rows - 16)
        return val[ro:ro + 16]
    rnd, val = tiles[-1]
    return val[rows - 16:rows]


def _finals(val, n_tiles, k_tiles, first_pass):
    return [((first_pass + (n + 1) * k_tiles - 1) // 4, val[:, n * 128:(n + 1) * 128])
            for n in range(n_tiles)]


def _recip(den):
    if RECIP == 0:
        return pl.reciprocal(den, approx=False)
    r = pl.reciprocal(den, approx=True)
    if RECIP == 1:
        r = r * (2.0 - den * r)
    return r


def _attention(q_s, k_s, v_s, a_s, last, rows, first, chain, ln_chunk):
    qs = (DH ** -0.5) * LOG2E
    dens = []
    pend = None
    rstd = None
    for c in range(rows // RA):
        r0 = c * RA
        if isinstance(last, list):
            sc = qs + jnp.minimum(jnp.abs(last[c]), 0.0)
        elif c >= chain:
            sc = qs + jnp.minimum(dens[c - chain], 0.0)
        else:
            sc = qs + jnp.minimum(jnp.abs(last[0:RA]), 0.0)
        if r0 % RC == 0:
            rstd = ln_chunk(r0 // RC)
            if rstd is not None:
                sc = sc + jnp.minimum(rstd[0:RA] if RA == RC else rstd[0:RA] + rstd[RA:2 * RA], 0.0)
        q = [q_s[j, r0:r0 + RA, :] * sc for j in range(NC)]
        ls = []
        for w in range(W):
            off = HALO + r0 - DIL * w
            p = q[0] * k_s[0, off:off + RA, :]
            for j in range(1, NC):
                p = p + q[j] * k_s[j, off:off + RA, :]
            if ROLL3:
                p = (p + pltpu.roll(p, 64, 1)) + (pltpu.roll(p, 32, 1) + pltpu.roll(p, 96, 1))
            else:
                p = p + pltpu.roll(p, 64, 1)
                p = p + pltpu.roll(p, 32, 1)
            if first and r0 < DIL * w:
                rows_i = r0 + lax.broadcasted_iota(jnp.int32, (RA, 128), 0)
                p = jnp.where(rows_i >= DIL * w, p, -1e9)
            ls.append(p)
        mx = jnp.maximum(jnp.maximum(jnp.maximum(ls[0], ls[1]), jnp.maximum(ls[2], ls[3])),
                         jnp.maximum(jnp.maximum(ls[4], ls[5]), jnp.maximum(ls[6], ls[7])))
        es = [jnp.exp2(l - mx) for l in ls]
        den = ((es[0] + es[1]) + (es[2] + es[3])) + ((es[4] + es[5]) + (es[6] + es[7]))
        inv = _recip(den)
        outs = []
        for j in range(NC):
            acc = None
            for w in range(W):
                off = HALO + r0 - DIL * w
                t = es[w] * v_s[j, off:off + RA, :]
                acc = t if acc is None else acc + t
            outs.append(acc * inv)
        dens.append(den if LINK == 0 else jnp.abs(outs[NC - 1]))
        if RA == 8 and c % 2 == 0:
            pend = outs
            continue
        if RA == 8:
            outs = [jnp.concatenate([a, b], axis=0) for a, b in zip(pend, outs)]
            r0 -= 8
        for j in range(NC):
            a_s[r0 // 2:r0 // 2 + 8, j * 128:(j + 1) * 128] = _pk(outs[j].astype(bf16))


def kernel(x_hbm, wqkv_hbm, wo_hbm, wg_hbm, wu_hbm, wd_hbm, o_hbm,
           x_v, o_v, wqkv_raw, wo_raw, wg_v, wu_v, wl_v, wd_v,
           wqkv_p, wo_p, wg_p, wu_p, wl_p, wd_p,
           wt0, wt1, wt2, wt3, wt4, zero_s,
           xn_s, q_s, k_s, v_s, a_s, sem, sem_b):
    wo_tmp = (wt0, wt1, wt2, wt3, wt4)
    zero_s[0] = 0
    NXP = len(XPIECES)

    def cp(src, dst, s):
        return pltpu.make_async_copy(src, dst, sem.at[s])

    def o_copy(r, n):
        return cp(o_v.at[pl.ds(r, n)], o_hbm.at[pl.ds(r, n)], 0)

    def fence():
        pl.semaphore_signal(sem_b, 1)
        pl.semaphore_wait(sem_b, 1)

    def gu_cp(ci, s):
        a, b = GU_CHUNKS[ci]
        return [cp(wg_hbm.at[a:b], wg_v.at[a:b], s), cp(wu_hbm.at[a:b], wu_v.at[a:b], s)]

    xp_cp = [cp(x_hbm.at[a:b], x_v.at[a:b], p) for p, (a, b) in enumerate(XPIECES)]
    g1 = [cp(wg_hbm.at[FM:F], wl_v.at[0:64], NXP), cp(wu_hbm.at[FM:F], wl_v.at[64:128], NXP)]
    g2 = gu_cp(0, NXP + 1)
    g3 = gu_cp(1, NXP + 2)
    g4 = gu_cp(2, NXP + 3) + [cp(wqkv_hbm.at[:, 0:2 * D], wqkv_raw.at[:, 0:2 * D], NXP + 3)]
    g5 = gu_cp(3, NXP + 4) + [cp(wqkv_hbm.at[:, 2 * D:3 * D], wqkv_raw.at[:, 2 * D:3 * D], NXP + 4),
                              cp(wd_hbm, wd_v, NXP + 4), cp(wo_hbm, wo_raw, NXP + 4),
                              cp(x_hbm.at[T0:T0 + T], x_v.at[T0:T0 + T], NXP + 4)]
    xr_cp = cp(x_hbm.at[T0 + T:S], x_v.at[T0 + T:S], 1)

    for c in xp_cp:
        c.start()
        fence()
    for g in (g1, g2, g3, g4, g5):
        for c in g:
            c.start()
        fence()

    k_s[:, 0:HALO, :] = jnp.zeros((NC, HALO, 128), f32)
    v_s[:, 0:HALO, :] = jnp.zeros((NC, HALO, 128), f32)

    gus = []

    def ffn_chunk(xn, a, b):
        wg = wg_v[a:b, :]
        wu = wu_v[a:b, :]
        wg_p[a // 2:b // 2, :] = _pk(wg)
        wu_p[a // 2:b // 2, :] = _pk(wu)
        g = lax.dot_general(xn, wg, NT_DIMS, preferred_element_type=f32)
        u = lax.dot_general(xn, wu, NT_DIMS, preferred_element_type=f32)
        gus.append((g, u))
        return _pk((_gelu(g) * u).astype(bf16))

    def proj(xn, w, dst, off):
        r = jnp.dot(xn, w, preferred_element_type=f32)
        for j in range(NC):
            dst[j, off:off + T0, :] = r[:, j * 128:(j + 1) * 128]
        return r

    def make_ln_chunk(r_next, outs, trig=None):
        def ln_chunk(c):
            if not LN_IN_CHAIN or c * RC >= T:
                return None
            if isinstance(r_next, int):
                xx = x_v[r_next + c * RC:r_next + (c + 1) * RC, :]
            else:
                xx = x_v[pl.ds(pl.multiple_of(r_next + c * RC, 16), RC), :]
            y, rstd = _ln(xx, None if trig is None else jnp.minimum(jnp.abs(trig[c]), 0.0))
            outs.append(y)
            return rstd
        return ln_chunk

    for (a, b), c in zip(XPIECES, xp_cp):
        c.wait()
        xn_s[a // 2:b // 2, :] = _pk(_ln(x_v[a:b, :])[0])
    hs = []
    for c in g1:
        c.wait()
    xn = _upk(xn_s[0:T0 // 2, :])
    wl = wl_v[...]
    wl_p[...] = _pk(wl)
    gu = lax.dot_general(xn, wl, NT_DIMS, preferred_element_type=f32)
    hl = _pk((_gelu(gu) * pltpu.roll(gu, 64, 1)).astype(bf16))
    for c in g2:
        c.wait()
    hs.append(ffn_chunk(xn, *GU_CHUNKS[0]))
    for c in g3:
        c.wait()
    hs.append(ffn_chunk(xn, *GU_CHUNKS[1]))
    for c in g4:
        c.wait()
    wq = _perm_cols(wqkv_raw, wqkv_p, 0)
    wk = _perm_cols(wqkv_raw, wqkv_p, 1)
    hs.append(ffn_chunk(xn, *GU_CHUNKS[2]))
    proj(xn, wq, q_s, 0)
    proj(xn, wk, k_s, HALO)
    for c in g5:
        c.wait()
    xr_cp.start()
    for j in range(NC):
        wo_tmp[j][0] = wo_raw[:, j * 128:(j + 1) * 128].astype(f32)
    wv = _perm_cols(wqkv_raw, wqkv_p, 2)
    a3, b3 = GU_CHUNKS[3]
    mid = a3 + MID
    na = MID // 128
    nb = (b3 - mid) // 128
    hs.append(ffn_chunk(xn, a3, mid))
    r = proj(xn, wv, v_s, HALO)
    hs.append(ffn_chunk(xn, mid, b3))
    h = _upk(jnp.concatenate(hs, axis=1))
    hl = _upk(hl)[:, 0:64]
    wd = wd_v[...]
    wd_p[...] = _pk(wd)
    tiles = (_finals(gus[-2][0], na, 5, 0) + _finals(gus[-2][1], na, 5, 5 * na) + _finals(r, 5, 5, 10 * na)
             + _finals(gus[-1][0], nb, 5, 10 * na + 25) + _finals(gus[-1][1], nb, 5, 10 * na + 25 + 5 * nb))
    hx = jnp.concatenate([h[:, 0:256], hl], axis=1)
    y = jnp.dot(hx, jnp.concatenate([wd[0:256, :], wd[FM:F, :]], axis=0), preferred_element_type=f32)
    tiles += _finals(y, 5, 3, 65)
    for kc, (lo, hi) in enumerate(((256, 768), (768, 1280), (1280, FM))):
        y = y + jnp.dot(h[:, lo:hi], wd[lo:hi, :], preferred_element_type=f32)
        tiles += _finals(y, 5, (hi - lo) // 128, 80 + 20 * kc)
    last = [_pick(tiles, T0, P_T0 + c * P_DT) for c in range(T0 // RA)]
    lnt = [_pick(tiles, T0, PLN_T0 + c * PLN_DT) for c in range(T // RC)]
    xn_parts = []
    _attention(q_s, k_s, v_s, a_s, last, T0, True, CHAIN0, make_ln_chunk(T0, xn_parts, lnt))
    wo = _perm_rows(wo_tmp, wo_p, zero_s[0])
    y = y + jnp.dot(_upk(a_s[0:T0 // 2, :]), wo, preferred_element_type=f32)
    o_v[0:T0, :] = (x_v[0:T0, :].astype(f32) + y).astype(bf16)
    if LN_IN_CHAIN:
        xn_s[0:T // 2, :] = _pk(jnp.concatenate(xn_parts, axis=0))
    else:
        xn_s[0:T // 2, :] = _pk(_ln(x_v[T0:T0 + T, :])[0])
    k_s[:, 0:HALO, :] = k_s[:, T0:T0 + HALO, :]
    v_s[:, 0:HALO, :] = v_s[:, T0:T0 + HALO, :]
    o_copy(0, T0).start()
    xr_cp.wait()

    def body(i, carry):
        r_cur = pl.multiple_of(T0 + i * T, 16)
        inext = jnp.minimum(i + 1, NL - 1)
        r_next = pl.multiple_of(T0 + inext * T, 16)
        xn = _upk(xn_s[0:T // 2, :])
        if not LN_IN_CHAIN:
            xn_next = _ln(x_v[pl.ds(r_next, T), :])[0]
        gu = lax.dot_general(xn, _upk(wl_p[...]), NT_DIMS, preferred_element_type=f32)
        hl = (_gelu(gu) * pltpu.roll(gu, 64, 1))[:, 0:64].astype(bf16)
        qkv = jnp.dot(xn, _upk(wqkv_p[...]), preferred_element_type=f32)
        for j in range(NC):
            q_s[j, 0:T, :] = qkv[:, j * 128:(j + 1) * 128]
            k_s[j, HALO:HALO + T, :] = qkv[:, D + j * 128:D + (j + 1) * 128]
            v_s[j, HALO:HALO + T, :] = qkv[:, 2 * D + j * 128:2 * D + (j + 1) * 128]
        last = qkv[T - RC:T, 3 * D - 128:3 * D]
        g = lax.dot_general(xn, _upk(wg_p[...]), NT_DIMS, preferred_element_type=f32)
        u = lax.dot_general(xn, _upk(wu_p[...]), NT_DIMS, preferred_element_type=f32)
        tiles = _finals(qkv, 15, 5, 4) + _finals(g, 13, 5, 79) + _finals(u, 13, 5, 144)
        last = [_pick(tiles, T, ATT_T0 + c * ATT_DT) for c in range(T // RA)]
        lnt = [_pick(tiles, T, LN_T0 + c * LN_DT) for c in range(T // RC)] if LN_TRIG else None
        xn_parts = []
        _attention(q_s, k_s, v_s, a_s, last, T, False, CHAIN, make_ln_chunk(r_next, xn_parts, lnt))
        if LN_IN_CHAIN:
            xn_next = jnp.concatenate(xn_parts, axis=0)
        h = (_gelu(g) * u).astype(bf16)
        y = jnp.dot(h, _upk(wd_p[0:FM // 2, :]), preferred_element_type=f32)
        y = y + jnp.dot(hl, _upk(wd_p[FM // 2:F // 2, :]), preferred_element_type=f32)
        y = y + jnp.dot(_upk(a_s[0:T // 2, :]), _upk(wo_p[...]), preferred_element_type=f32)
        o_v[pl.ds(r_cur, T), :] = (x_v[pl.ds(r_cur, T), :].astype(f32) + y).astype(bf16)
        xn_s[0:T // 2, :] = _pk(xn_next)
        k_s[:, 0:HALO, :] = k_s[:, T:T + HALO, :]
        v_s[:, 0:HALO, :] = v_s[:, T:T + HALO, :]
        o_copy(r_cur, T).start()
        return carry

    lax.fori_loop(0, NL, body, 0)
    o_copy(0, S).wait()


@jax.jit
def pallas_parallel_sum__sliding_local_dilated__geglu_ffn__prompt_kernel(
    A_x, A_wqkv, A_wo, B_x, B_w_gate, B_w_up, B_w_down):
    x = A_x.reshape(S, D)
    anyspec = pl.BlockSpec(memory_space=pl.ANY)
    out = pl.pallas_call(
        kernel,
        in_specs=[anyspec] * 6,
        out_specs=anyspec,
        out_shape=jax.ShapeDtypeStruct((S, D), bf16),
        scratch_shapes=[pltpu.VMEM((S, D), bf16),
                        pltpu.VMEM((S, D), bf16),
                        pltpu.VMEM((D, 3 * D), bf16),
                        pltpu.VMEM((D, D), bf16),
                        pltpu.VMEM((FM, D), bf16),
                        pltpu.VMEM((FM, D), bf16),
                        pltpu.VMEM((128, D), bf16),
                        pltpu.VMEM((F, D), bf16),
                        pltpu.VMEM((D // 2, 3 * D), u32),
                        pltpu.VMEM((D // 2, D), u32),
                        pltpu.VMEM((FM // 2, D), u32),
                        pltpu.VMEM((FM // 2, D), u32),
                        pltpu.VMEM((64, D), u32),
                        pltpu.VMEM((F // 2, D), u32),
                        pltpu.VMEM((2, D, 128), f32),
                        pltpu.VMEM((2, D, 128), f32),
                        pltpu.VMEM((2, D, 128), f32),
                        pltpu.VMEM((2, D, 128), f32),
                        pltpu.VMEM((2, D, 128), f32),
                        pltpu.SMEM((1,), jnp.int32),
                        pltpu.VMEM((TM // 2, D), u32),
                        pltpu.VMEM((NC, TM, 128), f32),
                        pltpu.VMEM((NC, TM + HALO, 128), f32),
                        pltpu.VMEM((NC, TM + HALO, 128), f32),
                        pltpu.VMEM((TM // 2, D), u32),
                        pltpu.SemaphoreType.DMA((len(XPIECES) + 5,)),
                        pltpu.SemaphoreType.REGULAR],
        compiler_params=pltpu.CompilerParams(vmem_limit_bytes=100 * 1024 * 1024),
    )(x, A_wqkv, A_wo, B_w_gate.T, B_w_up.T, B_w_down)
    return out.reshape(1, S, D)
```

```python
import jax
import jax.numpy as jnp
from jax import lax
import jax.experimental.pallas as pl
import jax.experimental.pallas.tpu as pltpu

S, D, F = 2048, 640, 1728
H, DH, W, DIL = 32, 20, 8, 2
T0 = 528
T = 304
NL = (S - T0) // T
assert T0 + NL * T == S
XPIECES = ((0, 144), (144, 272), (272, 400), (400, 528))
HALO = 16
NC = D // 128
RC = 16
FM = 1664
LOG2E = 1.4426950408889634
NT_DIMS = (((1,), (1,)), ((), ()))
ATT_T0 = 19.9
ATT_DT = 1.2
LN_T0 = 8.5
LN_DT = 0.58
DTRIG = ((0, 0), (0, 1), (1, 0), (1, 1), (2, 0))
P_T0 = 0.7
P_DT = 0.7
P_N = 16
P_T1 = 20.5
P_DT1 = 0.72
PLN_T0 = 12.5
PLN_DT = 0.4
PLN_OFF = 14
OPIECES = (2, 3, 4)
f32 = jnp.float32
bf16 = jnp.bfloat16
u32 = jnp.uint32


def _pk(x):
    return pltpu.bitcast(x, u32)


def _upk(x):
    return pltpu.bitcast(x, bf16)


def _dot(a, b):
    return jnp.dot(a, b, preferred_element_type=f32)


def _dot_nt(a, b):
    return lax.dot_general(a, b, NT_DIMS, preferred_element_type=f32)


def _zero(v):
    return jnp.minimum(jnp.abs(v), 0.0)


def _gelu(x):
    c = 0.7978845608028654
    inner = x * (c + (c * 0.044715) * (x * x))
    return (0.5 * x) * (1.0 + jnp.tanh(inner))


def _ln(x, z=None):
    x = x.astype(f32)
    t = x[:, 0:128] if z is None else z + x[:, 0:128]
    for j in range(1, NC):
        t = t + x[:, j * 128:(j + 1) * 128]
    m = jnp.sum(t, axis=-1, keepdims=True) * (1.0 / D)
    xc = x - m
    var = jnp.mean(xc * xc, axis=-1, keepdims=True)
    rstd = lax.rsqrt(var + 1e-5)
    return (xc * rstd).astype(bf16), rstd


def _perm_cols(src_ref, dst_ref, p):
    R = D // 2
    lane = lax.broadcasted_iota(jnp.int32, (8, 128), 1)
    outs = []
    for j in range(NC):
        rel = (lane + (128 - 4 * j)) & 127
        h = (13 * (rel >> 2)) & 31
        c = jnp.tile(20 * h + 4 * j + (rel & 3), (R // 8, 1))
        idx = jnp.tile((20 * (lane & 31) + 4 * j + (lane >> 5)) & 127, (R // 8, 1))
        w = [_pk(src_ref[:, p * D + i * 128: p * D + (i + 1) * 128]) for i in range(NC)]
        s = w[4]
        for i in (3, 2, 1, 0):
            s = jnp.where(c < 128 * (i + 1), w[i], s)
        g = jnp.take_along_axis(s, idx, axis=1)
        dst_ref[:, p * D + j * 128: p * D + (j + 1) * 128] = g
        outs.append(_upk(g))
    return jnp.concatenate(outs, axis=1)


def _perm_rows(tmp_ref, dst_ref):
    cols = []
    for j in range(NC):
        blk = jnp.concatenate(
            [tmp_ref[j, pl.ds(d, H, stride=DH), :].astype(bf16) for d in range(DH)], axis=0)
        dst_ref[:, j * 128:(j + 1) * 128] = _pk(blk)
        cols.append(blk)
    return jnp.concatenate(cols, axis=1)


class _Sched:
    def __init__(self, rows, first_pass):
        self.rows, self.p, self.tiles = rows, first_pass, []

    def add(self, val, k_tiles):
        for n in range(val.shape[1] // 128):
            self.p += k_tiles
            self.tiles.append(((self.p - 1) // 4, val[:, n * 128:(n + 1) * 128]))
        return val

    def pick(self, t):
        for rnd, val in self.tiles:
            if rnd + 1 <= t:
                continue
            ro = min(8 * int(max(t - rnd, 0.0) * self.rows / 8), self.rows - RC)
            return val[ro:ro + RC]
        return self.tiles[-1][1][self.rows - RC:self.rows]


def _attention(q_s, k_s, v_s, a_s, trig, rows, first, ln_chunk):
    qs = (DH ** -0.5) * LOG2E
    for c in range(rows // RC):
        r0 = c * RC
        sc = qs + _zero(trig[c])
        rstd = ln_chunk(c)
        if rstd is not None:
            sc = sc + jnp.minimum(rstd, 0.0)
        q = [q_s[j, r0:r0 + RC, :] * sc for j in range(NC)]
        ls = []
        for w in range(W):
            off = HALO + r0 - DIL * w
            p = q[0] * k_s[0, off:off + RC, :]
            for j in range(1, NC):
                p = p + q[j] * k_s[j, off:off + RC, :]
            p = p + pltpu.roll(p, 64, 1)
            p = p + pltpu.roll(p, 32, 1)
            if first and r0 < DIL * w:
                rows_i = r0 + lax.broadcasted_iota(jnp.int32, (RC, 128), 0)
                p = jnp.where(rows_i >= DIL * w, p, -1e9 * LOG2E)
            ls.append(p)
        mx = jnp.maximum(jnp.maximum(jnp.maximum(ls[0], ls[1]), jnp.maximum(ls[2], ls[3])),
                         jnp.maximum(jnp.maximum(ls[4], ls[5]), jnp.maximum(ls[6], ls[7])))
        es = [jnp.exp2(l - mx) for l in ls]
        den = ((es[0] + es[1]) + (es[2] + es[3])) + ((es[4] + es[5]) + (es[6] + es[7]))
        inv = pl.reciprocal(den, approx=True)
        inv = inv * (2.0 - den * inv)
        for j in range(NC):
            acc = None
            for w in range(W):
                off = HALO + r0 - DIL * w
                t = es[w] * v_s[j, off:off + RC, :]
                acc = t if acc is None else acc + t
            a_s[r0 // 2:(r0 + RC) // 2, j * 128:(j + 1) * 128] = _pk((acc * inv).astype(bf16))


def _kernel(x_hbm, wqkv_hbm, wo_hbm, wg_hbm, wu_hbm, wd_hbm, o_hbm,
            x_v, o_v, wqkv_raw, wo_raw, wg_v, wu_v, wl_v, wd_v,
            wqkv_p, wo_p, wg_p, wu_p, wl_p, wd_p, wo_tmp,
            xn_s, q_s, k_s, v_s, a_s, sem, sem_b):
    NXP = len(XPIECES)

    def cp(src, dst, s):
        return pltpu.make_async_copy(src, dst, sem.at[s])

    def fence():
        pl.semaphore_signal(sem_b, 1)
        pl.semaphore_wait(sem_b, 1)

    def rows_cp(src, dst, a, b, s):
        return cp(src.at[a:b], dst.at[a:b], s)

    xp_cp = [rows_cp(x_hbm, x_v, a, b, p) for p, (a, b) in enumerate(XPIECES)]
    g1 = [cp(wg_hbm.at[FM:F], wl_v.at[0:64], NXP), cp(wu_hbm.at[FM:F], wl_v.at[64:128], NXP)]
    g2 = [rows_cp(wg_hbm, wg_v, 0, 256, NXP + 1), rows_cp(wu_hbm, wu_v, 0, 256, NXP + 1)]
    g3 = [rows_cp(wg_hbm, wg_v, 256, 768, NXP + 2), rows_cp(wu_hbm, wu_v, 256, 768, NXP + 2)]
    g4 = [rows_cp(wg_hbm, wg_v, 768, 896, NXP + 3), cp(wqkv_hbm, wqkv_raw, NXP + 3)]
    g5 = [rows_cp(wg_hbm, wg_v, 896, FM, NXP + 4), rows_cp(wu_hbm, wu_v, 768, FM, NXP + 4),
          cp(wd_hbm, wd_v, NXP + 4), cp(wo_hbm, wo_raw, NXP + 4),
          rows_cp(x_hbm, x_v, T0, T0 + T, NXP + 4)]
    xr_cp = rows_cp(x_hbm, x_v, T0 + T, S, 1)

    for c in xp_cp:
        c.start()
        fence()
    for g in (g1, g2, g3, g4, g5):
        for c in g:
            c.start()
        fence()

    k_s[:, 0:HALO, :] = jnp.zeros((NC, HALO, 128), f32)
    v_s[:, 0:HALO, :] = jnp.zeros((NC, HALO, 128), f32)

    def gate(xn, a, b):
        wg = wg_v[a:b, :]
        wg_p[a // 2:b // 2, :] = _pk(wg)
        return _dot_nt(xn, wg)

    def up(xn, a, b):
        wu = wu_v[a:b, :]
        wu_p[a // 2:b // 2, :] = _pk(wu)
        return _dot_nt(xn, wu)

    def act(g, u):
        return _pk((_gelu(g) * u).astype(bf16))

    def put(r, dst, off, rows, c0=0):
        for j in range(NC):
            dst[j, off:off + rows, :] = r[:, c0 + j * 128:c0 + (j + 1) * 128]

    def make_ln_chunk(r_next, outs, trig, off=0):
        def ln_chunk(c):
            c = c - off
            if c < 0 or c * RC >= T:
                return None
            if isinstance(r_next, int):
                xx = x_v[r_next + c * RC:r_next + (c + 1) * RC, :]
            else:
                xx = x_v[pl.ds(pl.multiple_of(r_next + c * RC, 16), RC), :]
            y, rstd = _ln(xx, _zero(trig[c]))
            outs.append(_pk(y))
            return rstd
        return ln_chunk

    def write_out(r, rows, y, split):
        if not split:
            o_v[pl.ds(r, rows), :] = (x_v[pl.ds(r, rows), :].astype(f32) + y).astype(bf16)
            cp(o_v.at[pl.ds(r, rows)], o_hbm.at[pl.ds(r, rows)], 0).start()
            return
        lo = 0
        for j in range(NC):
            cs = slice(j * 128, (j + 1) * 128)
            o_v[pl.ds(r, rows), cs] = (x_v[pl.ds(r, rows), cs].astype(f32) + y[:, cs]).astype(bf16)
            if j in OPIECES:
                ps = slice(lo, (j + 1) * 128)
                lo = (j + 1) * 128
                cp(o_v.at[pl.ds(r, rows), ps], o_hbm.at[pl.ds(r, rows), ps], 0).start()

    for (a, b), c in zip(XPIECES, xp_cp):
        c.wait()
        xn_s[a // 2:b // 2, :] = _pk(_ln(x_v[a:b, :])[0])
    hs = []
    for c in g1:
        c.wait()
    xn = _upk(xn_s[0:T0 // 2, :])
    wl = wl_v[...]
    wl_p[...] = _pk(wl)
    gu = _dot_nt(xn, wl)
    hl = act(gu, pltpu.roll(gu, 64, 1))
    for c in g2:
        c.wait()
    g0, u0 = gate(xn, 0, 256), up(xn, 0, 256)
    hs.append(act(g0, u0))
    for c in g3:
        c.wait()
    g1_, u1 = gate(xn, 256, 768), up(xn, 256, 768)
    hs.append(act(g1_, u1))
    for c in g4:
        c.wait()
    wq = _perm_cols(wqkv_raw, wqkv_p, 0)
    wk = _perm_cols(wqkv_raw, wqkv_p, 1)
    wv = _perm_cols(wqkv_raw, wqkv_p, 2)
    ga = gate(xn, 768, 896)
    put(_dot(xn, wq), q_s, 0, T0)
    put(_dot(xn, wk), k_s, HALO, T0)
    put(_dot(xn, wv), v_s, HALO, T0)
    for c in g5:
        c.wait()
    xr_cp.start()
    sch = _Sched(T0, 0)
    wd = wd_v[...]
    wd_p[...] = _pk(wd)
    hx = jnp.concatenate([_upk(hs[0]), _upk(hl)[:, 0:64]], axis=1)
    y = sch.add(_dot(hx, jnp.concatenate([wd[0:256, :], wd[FM:F, :]], axis=0)), 3)
    gb = sch.add(gate(xn, 896, FM), 5)
    ub = sch.add(up(xn, 768, FM), 5)
    hs.append(act(jnp.concatenate([ga, gb], axis=1), ub))
    h = _upk(jnp.concatenate(hs, axis=1))
    for lo, hi in ((256, 768), (768, 1280), (1280, FM)):
        y = sch.add(y + _dot(h[:, lo:hi], wd[lo:hi, :]), (hi - lo) // 128)
    trig = [sch.pick(P_T0 + c * P_DT) for c in range(P_N)]
    trig += [sch.pick(P_T1 + c * P_DT1) for c in range(T0 // RC - P_N)]
    lnt = [sch.pick(PLN_T0 + c * PLN_DT) for c in range(T // RC)]
    xn_parts = []
    _attention(q_s, k_s, v_s, a_s, trig, T0, True, make_ln_chunk(T0, xn_parts, lnt, PLN_OFF))
    for j in range(NC):
        for b in range(4):
            rb = D // 4
            wo_tmp[j, b * rb:(b + 1) * rb, :] = (
                wo_raw[b * rb:(b + 1) * rb, j * 128:(j + 1) * 128].astype(f32))
    wo = _perm_rows(wo_tmp, wo_p)
    y = y + _dot(_upk(a_s[0:T0 // 2, :]), wo)
    write_out(0, T0, y, False)
    xn_s[0:T // 2, :] = jnp.concatenate(xn_parts, axis=0)
    k_s[:, 0:HALO, :] = k_s[:, T0:T0 + HALO, :]
    v_s[:, 0:HALO, :] = v_s[:, T0:T0 + HALO, :]
    xr_cp.wait()

    def body(i, carry):
        r_cur = pl.multiple_of(T0 + i * T, 16)
        inext = jnp.minimum(i + 1, NL - 1)
        r_next = pl.multiple_of(T0 + inext * T, 16)
        xn = _upk(xn_s[0:T // 2, :])
        sch = _Sched(T, -1)
        put(sch.add(_dot(xn, _upk(wqkv_p[:, 0:D])), 5), q_s, 0, T)
        gu = sch.add(_dot_nt(xn, _upk(wl_p[...])), 5)
        kv = sch.add(_dot(xn, _upk(wqkv_p[:, D:3 * D])), 5)
        put(kv, k_s, HALO, T)
        put(kv, v_s, HALO, T, D)
        hl = (_gelu(gu) * pltpu.roll(gu, 64, 1))[:, 0:64].astype(bf16)
        g = sch.add(_dot_nt(xn, _upk(wg_p[...])), 5)
        u = sch.add(_dot_nt(xn, _upk(wu_p[...])), 5)
        h = (_gelu(g) * u).astype(bf16)
        y = _dot(h, _upk(wd_p[0:FM // 2, :]))
        y = y + _dot(hl, _upk(wd_p[FM // 2:F // 2, :]))
        trig = [sch.pick(ATT_T0 + c * ATT_DT) for c in range(T // RC - len(DTRIG))]
        for n, fr in DTRIG:
            ro = min(8 * int(fr * T / 8), T - RC)
            trig.append(y[ro:ro + RC, n * 128:(n + 1) * 128])
        lnt = [sch.pick(LN_T0 + c * LN_DT) for c in range(T // RC)]
        xn_parts = []
        _attention(q_s, k_s, v_s, a_s, trig, T, False, make_ln_chunk(r_next, xn_parts, lnt))
        y = y + _dot(_upk(a_s[0:T // 2, :]), _upk(wo_p[...]))
        write_out(r_cur, T, y, True)
        xn_s[0:T // 2, :] = jnp.concatenate(xn_parts, axis=0)
        k_s[:, 0:HALO, :] = k_s[:, T:T + HALO, :]
        v_s[:, 0:HALO, :] = v_s[:, T:T + HALO, :]
        return carry

    lax.fori_loop(0, NL, body, 0)
    cp(o_v, o_hbm, 0).wait()


@jax.jit
def pallas_parallel_sum__sliding_local_dilated__geglu_ffn__prompt_kernel(
    A_x: jax.Array,
    A_wqkv: jax.Array,
    A_wo: jax.Array,
    B_x: jax.Array,
    B_w_gate: jax.Array,
    B_w_up: jax.Array,
    B_w_down: jax.Array,
):
    del B_x
    anyspec = pl.BlockSpec(memory_space=pl.ANY)
    out = pl.pallas_call(
        _kernel,
        in_specs=[anyspec] * 6,
        out_specs=anyspec,
        out_shape=jax.ShapeDtypeStruct((S, D), bf16),
        scratch_shapes=[pltpu.VMEM((S, D), bf16),
                        pltpu.VMEM((S, D), bf16),
                        pltpu.VMEM((D, 3 * D), bf16),
                        pltpu.VMEM((D, D), bf16),
                        pltpu.VMEM((FM, D), bf16),
                        pltpu.VMEM((FM, D), bf16),
                        pltpu.VMEM((128, D), bf16),
                        pltpu.VMEM((F, D), bf16),
                        pltpu.VMEM((D // 2, 3 * D), u32),
                        pltpu.VMEM((D // 2, D), u32),
                        pltpu.VMEM((FM // 2, D), u32),
                        pltpu.VMEM((FM // 2, D), u32),
                        pltpu.VMEM((64, D), u32),
                        pltpu.VMEM((F // 2, D), u32),
                        pltpu.VMEM((NC, D, 128), f32),
                        pltpu.VMEM((T0 // 2, D), u32),
                        pltpu.VMEM((NC, T0, 128), f32),
                        pltpu.VMEM((NC, T0 + HALO, 128), f32),
                        pltpu.VMEM((NC, T0 + HALO, 128), f32),
                        pltpu.VMEM((T0 // 2, D), u32),
                        pltpu.SemaphoreType.DMA((len(XPIECES) + 5,)),
                        pltpu.SemaphoreType.REGULAR],
        compiler_params=pltpu.CompilerParams(vmem_limit_bytes=100 * 1024 * 1024,
                                             disable_bounds_checks=True,
                                             disable_semaphore_checks=True),
    )(A_x.reshape(S, D), A_wqkv, A_wo, B_w_gate.T, B_w_up.T, B_w_down)
    return out.reshape(1, S, D)
```

```python
import jax
import jax.numpy as jnp
from jax import lax
import jax.experimental.pallas as pl
import jax.experimental.pallas.tpu as pltpu

S, D, F = 2048, 640, 1728
H, DH, W, DIL = 32, 20, 8, 2
T0 = 512
T = 384
NL = (S - T0) // T
assert T0 + NL * T == S
XPIECES = ((0, 128), (128, 256), (256, 384), (384, 512))
HALO = 16
NC = D // 128
RC = 16
FM = 1664
LOG2E = 1.4426950408889634
NT_DIMS = (((1,), (1,)), ((), ()))
ATT_T0 = 19.9
ATT_DT = 0.95
LN_T0 = 8.5
LN_DT = 0.46
DTRIG = ((0, 0), (0, 1), (1, 0), (1, 1), (2, 0), (2, 1))
P_T0 = 0.2
P_DT = 0.771
P_N = 15
P_T1 = 19.0
P_DT1 = 0.469
PLN_T0 = 0.3
PLN_DT = 0.771
PLN_OFF = 8
PLN_R = 1.0
WO5A = True
WO_NB = 4
WO_T0 = 0.3
WO_DT = 0.17
OPIECES = (2, 3, 4)
f32 = jnp.float32
bf16 = jnp.bfloat16
u32 = jnp.uint32


def _pk(x):
    return pltpu.bitcast(x, u32)


def _upk(x):
    return pltpu.bitcast(x, bf16)


def _dot(a, b):
    return jnp.dot(a, b, preferred_element_type=f32)


def _dot_nt(a, b):
    return lax.dot_general(a, b, NT_DIMS, preferred_element_type=f32)


def _zero(v):
    return jnp.minimum(jnp.abs(v), 0.0)


def _gelu(x):
    c = 0.7978845608028654
    inner = x * (c + (c * 0.044715) * (x * x))
    return (0.5 * x) * (1.0 + jnp.tanh(inner))


def _ln(x, z=None):
    x = x.astype(f32)
    t = x[:, 0:128] if z is None else z + x[:, 0:128]
    for j in range(1, NC):
        t = t + x[:, j * 128:(j + 1) * 128]
    m = jnp.sum(t, axis=-1, keepdims=True) * (1.0 / D)
    xc = x - m
    var = jnp.mean(xc * xc, axis=-1, keepdims=True)
    rstd = lax.rsqrt(var + 1e-5)
    return (xc * rstd).astype(bf16), rstd


def _perm_cols(src_ref, dst_ref, p):
    R = D // 2
    lane = lax.broadcasted_iota(jnp.int32, (8, 128), 1)
    outs = []
    for j in range(NC):
        rel = (lane + (128 - 4 * j)) & 127
        h = (13 * (rel >> 2)) & 31
        c = jnp.tile(20 * h + 4 * j + (rel & 3), (R // 8, 1))
        idx = jnp.tile((20 * (lane & 31) + 4 * j + (lane >> 5)) & 127, (R // 8, 1))
        w = [_pk(src_ref[:, p * D + i * 128: p * D + (i + 1) * 128]) for i in range(NC)]
        s = w[4]
        for i in (3, 2, 1, 0):
            s = jnp.where(c < 128 * (i + 1), w[i], s)
        g = jnp.take_along_axis(s, idx, axis=1)
        dst_ref[:, p * D + j * 128: p * D + (j + 1) * 128] = g
        outs.append(_upk(g))
    return jnp.concatenate(outs, axis=1)


def _perm_rows(tmp_ref, dst_ref):
    cols = []
    for j in range(NC):
        blk = jnp.concatenate(
            [tmp_ref[j, pl.ds(d, H, stride=DH), :].astype(bf16) for d in range(DH)], axis=0)
        dst_ref[:, j * 128:(j + 1) * 128] = _pk(blk)
        cols.append(blk)
    return jnp.concatenate(cols, axis=1)


class _Sched:
    def __init__(self, rows, first_pass):
        self.rows, self.p, self.tiles = rows, first_pass, []

    def add(self, val, k_tiles):
        for n in range(val.shape[1] // 128):
            self.p += k_tiles
            self.tiles.append(((self.p - 1) // 4, val[:, n * 128:(n + 1) * 128]))
        return val

    def pick(self, t):
        for rnd, val in self.tiles:
            if rnd + 1 <= t:
                continue
            ro = min(8 * int(max(t - rnd, 0.0) * self.rows / 8), self.rows - RC)
            return val[ro:ro + RC]
        return self.tiles[-1][1][self.rows - RC:self.rows]


def _attention(q_s, k_s, v_s, a_s, trig, rows, first, ln_chunk):
    qs = (DH ** -0.5) * LOG2E
    for c in range(rows // RC):
        r0 = c * RC
        sc = qs + _zero(trig[c])
        rstd = ln_chunk(c)
        if rstd is not None:
            sc = sc + jnp.minimum(rstd, 0.0)
        q = [q_s[j, r0:r0 + RC, :] * sc for j in range(NC)]
        ls = []
        for w in range(W):
            off = HALO + r0 - DIL * w
            p = q[0] * k_s[0, off:off + RC, :]
            for j in range(1, NC):
                p = p + q[j] * k_s[j, off:off + RC, :]
            p = p + pltpu.roll(p, 64, 1)
            p = p + pltpu.roll(p, 32, 1)
            if first and r0 < DIL * w:
                rows_i = r0 + lax.broadcasted_iota(jnp.int32, (RC, 128), 0)
                p = jnp.where(rows_i >= DIL * w, p, -1e9 * LOG2E)
            ls.append(p)
        mx = jnp.maximum(jnp.maximum(jnp.maximum(ls[0], ls[1]), jnp.maximum(ls[2], ls[3])),
                         jnp.maximum(jnp.maximum(ls[4], ls[5]), jnp.maximum(ls[6], ls[7])))
        es = [jnp.exp2(l - mx) for l in ls]
        den = ((es[0] + es[1]) + (es[2] + es[3])) + ((es[4] + es[5]) + (es[6] + es[7]))
        inv = pl.reciprocal(den, approx=True)
        inv = inv * (2.0 - den * inv)
        for j in range(NC):
            acc = None
            for w in range(W):
                off = HALO + r0 - DIL * w
                t = es[w] * v_s[j, off:off + RC, :]
                acc = t if acc is None else acc + t
            a_s[r0 // 2:(r0 + RC) // 2, j * 128:(j + 1) * 128] = _pk((acc * inv).astype(bf16))


def _kernel(x_hbm, wqkv_hbm, wo_hbm, wg_hbm, wu_hbm, wd_hbm, o_hbm,
            x_v, o_v, wqkv_raw, wo_raw, wg_v, wu_v, wl_v, wd_v,
            wqkv_p, wo_p, wg_p, wu_p, wl_p, wd_p, wo_tmp, y_s, g_s,
            xn_s, q_s, k_s, v_s, a_s, sem, sem_b):
    NXP = len(XPIECES)

    def cp(src, dst, s):
        return pltpu.make_async_copy(src, dst, sem.at[s])

    def fence():
        pl.semaphore_signal(sem_b, 1)
        pl.semaphore_wait(sem_b, 1)

    def rows_cp(src, dst, a, b, s):
        return cp(src.at[a:b], dst.at[a:b], s)

    xp_cp = [rows_cp(x_hbm, x_v, a, b, p) for p, (a, b) in enumerate(XPIECES)]
    g1 = [cp(wg_hbm.at[FM:F], wl_v.at[0:64], NXP), cp(wu_hbm.at[FM:F], wl_v.at[64:128], NXP),
          cp(wg_hbm.at[1536:FM, 0:512], wg_v.at[1536:FM, 0:512], NXP)]
    g2 = [rows_cp(wg_hbm, wg_v, 0, 256, NXP + 1), rows_cp(wu_hbm, wu_v, 0, 256, NXP + 1)]
    g3 = [rows_cp(wg_hbm, wg_v, 256, 768, NXP + 2), rows_cp(wu_hbm, wu_v, 256, 768, NXP + 2)]
    g4 = [rows_cp(wg_hbm, wg_v, 768, 896, NXP + 3), cp(wqkv_hbm, wqkv_raw, NXP + 3)]
    g5 = [rows_cp(wg_hbm, wg_v, 896, 1024, NXP + 4), cp(wd_hbm, wd_v, NXP + 4),
          cp(wo_hbm, wo_raw, NXP + 4)]
    g6 = [rows_cp(wg_hbm, wg_v, 1024, 1536, NXP + 5), rows_cp(wu_hbm, wu_v, 768, FM, NXP + 5),
          cp(wg_hbm.at[1536:FM, 512:D], wg_v.at[1536:FM, 512:D], NXP + 5),
          rows_cp(x_hbm, x_v, T0, T0 + T, NXP + 5)]
    xr_cp = rows_cp(x_hbm, x_v, T0 + T, S, 1)

    for c in xp_cp:
        c.start()
        fence()
    for g in (g1, g2, g3, g4, g5, g6):
        for c in g:
            c.start()
        fence()

    k_s[:, 0:HALO, :] = jnp.zeros((NC, HALO, 128), f32)
    v_s[:, 0:HALO, :] = jnp.zeros((NC, HALO, 128), f32)

    def gate(xn, a, b):
        wg = wg_v[a:b, :]
        wg_p[a // 2:b // 2, :] = _pk(wg)
        return _dot_nt(xn, wg)

    def up(xn, a, b):
        wu = wu_v[a:b, :]
        wu_p[a // 2:b // 2, :] = _pk(wu)
        return _dot_nt(xn, wu)

    def act(g, u):
        return _pk((_gelu(g) * u).astype(bf16))

    def put(r, dst, off, rows, c0=0):
        for j in range(NC):
            dst[j, off:off + rows, :] = r[:, c0 + j * 128:c0 + (j + 1) * 128]

    def make_ln_chunk(r_next, outs, trig, link=None):
        n = T // RC
        link = list(range(n)) if link is None else link

        def one(c):
            if isinstance(r_next, int):
                xx = x_v[r_next + c * RC:r_next + (c + 1) * RC, :]
            else:
                xx = x_v[pl.ds(pl.multiple_of(r_next + c * RC, 16), RC), :]
            y, rstd = _ln(xx, _zero(trig[c]))
            outs.append(_pk(y))
            return rstd

        def ln_chunk(a):
            tot = None
            for c in range(n):
                if link[c] == a:
                    r = one(c)
                    tot = r if tot is None else tot + r
            return tot
        return ln_chunk

    def write_out(r, rows, y, split):
        if not split:
            o_v[pl.ds(r, rows), :] = (x_v[pl.ds(r, rows), :].astype(f32) + y).astype(bf16)
            cp(o_v.at[pl.ds(r, rows)], o_hbm.at[pl.ds(r, rows)], 0).start()
            return
        lo = 0
        for j in range(NC):
            cs = slice(j * 128, (j + 1) * 128)
            o_v[pl.ds(r, rows), cs] = (x_v[pl.ds(r, rows), cs].astype(f32) + y[:, cs]).astype(bf16)
            if j in OPIECES:
                ps = slice(lo, (j + 1) * 128)
                lo = (j + 1) * 128
                cp(o_v.at[pl.ds(r, rows), ps], o_hbm.at[pl.ds(r, rows), ps], 0).start()

    def prologue():
        for (a, b), c in zip(XPIECES, xp_cp):
            c.wait()
            xn_s[a // 2:b // 2, :] = _pk(_ln(x_v[a:b, :])[0])
        hs = []
        for c in g1:
            c.wait()
        xn = _upk(xn_s[0:T0 // 2, :])
        wl = wl_v[...]
        wl_p[...] = _pk(wl)
        gu = _dot_nt(xn, wl)
        hl = act(gu, pltpu.roll(gu, 64, 1))
        wga = wg_v[1536:FM, 0:512]
        wg_p[768:FM // 2, 0:512] = _pk(wga)
        g_s[...] = _dot_nt(xn[:, 0:512], wga)
        for c in g2:
            c.wait()
        g0, u0 = gate(xn, 0, 256), up(xn, 0, 256)
        hs.append(act(g0, u0))
        for c in g3:
            c.wait()
        g1_, u1 = gate(xn, 256, 768), up(xn, 256, 768)
        hs.append(act(g1_, u1))
        for c in g4:
            c.wait()
        wq = _perm_cols(wqkv_raw, wqkv_p, 0)
        wk = _perm_cols(wqkv_raw, wqkv_p, 1)
        wv = _perm_cols(wqkv_raw, wqkv_p, 2)
        ga = gate(xn, 768, 896)
        put(_dot(xn, wq), q_s, 0, T0)
        put(_dot(xn, wk), k_s, HALO, T0)
        put(_dot(xn, wv), v_s, HALO, T0)
        for c in g5:
            c.wait()
        wd0 = jnp.concatenate([wd_v[0:256, :], wd_v[FM:F, :]], axis=0)
        wd_p[0:128, :] = _pk(wd0[0:256])
        wd_p[FM // 2:F // 2, :] = _pk(wd0[256:320])
        hx = jnp.concatenate([_upk(hs[0]), _upk(hl)[:, 0:64]], axis=1)
        sch = _Sched(T0, 0)
        y = sch.add(_dot(hx, wd0), 3)
        y_s[...] = y
        ga2 = sch.add(gate(xn, 896, 1024), 5)
        if WO5A:
            rb = D // WO_NB
            for j in range(NC):
                for b in range(WO_NB):
                    z = jnp.tile(_zero(sch.pick(WO_T0 + (j * WO_NB + b) * WO_DT)), (rb // RC, 1))
                    wo_tmp[j, b * rb:(b + 1) * rb, :] = (
                        wo_raw[b * rb:(b + 1) * rb, j * 128:(j + 1) * 128].astype(f32) + z)
        for c in g6:
            c.wait()
        xr_cp.start()
        sch = _Sched(T0, 0)
        wd = wd_v[256:FM, :]
        wd_p[128:FM // 2, :] = _pk(wd)
        y = sch.add(y_s[...] + _dot(_upk(hs[1]), wd[0:512, :]), 4)
        gb = sch.add(gate(xn, 1024, 1536), 5)
        wgb = wg_v[1536:FM, 512:D]
        wg_p[768:FM // 2, 512:D] = _pk(wgb)
        gc = sch.add(g_s[...] + _dot_nt(xn[:, 512:D], wgb), 1)
        ub = sch.add(up(xn, 768, FM), 5)
        hs.append(act(jnp.concatenate([ga, ga2, gb, gc], axis=1), ub))
        h = _upk(jnp.concatenate(hs, axis=1))
        for lo, hi in ((768, 1280), (1280, FM)):
            y = sch.add(y + _dot(h[:, lo:hi], wd[lo - 256:hi - 256, :]), (hi - lo) // 128)
        trig = [sch.pick(P_T0 + c * P_DT) for c in range(P_N)]
        trig += [sch.pick(P_T1 + c * P_DT1) for c in range(T0 // RC - P_N)]
        lnt = [sch.pick(PLN_T0 + c * PLN_DT) for c in range(T // RC)]
        xn_parts = []
        _attention(q_s, k_s, v_s, a_s, trig, T0, True, make_ln_chunk(T0, xn_parts, lnt, [min(T0 // RC - 1, PLN_OFF + int(c * PLN_R)) for c in range(T // RC)]))
        if not WO5A:
            for j in range(NC):
                wo_tmp[j] = wo_raw[:, j * 128:(j + 1) * 128].astype(f32)
        wo = _perm_rows(wo_tmp, wo_p)
        y = y + _dot(_upk(a_s[0:T0 // 2, :]), wo)
        write_out(0, T0, y, False)
        xn_s[0:T // 2, :] = jnp.concatenate(xn_parts, axis=0)
        k_s[:, 0:HALO, :] = k_s[:, T0:T0 + HALO, :]
        v_s[:, 0:HALO, :] = v_s[:, T0:T0 + HALO, :]
        xr_cp.wait()

    def body(i):
        r_cur = pl.multiple_of(T0 + i * T, 16)
        inext = jnp.minimum(i + 1, NL - 1)
        r_next = pl.multiple_of(T0 + inext * T, 16)
        xn = _upk(xn_s[0:T // 2, :])
        sch = _Sched(T, -1)
        put(sch.add(_dot(xn, _upk(wqkv_p[:, 0:D])), 5), q_s, 0, T)
        gu = sch.add(_dot_nt(xn, _upk(wl_p[...])), 5)
        kv = sch.add(_dot(xn, _upk(wqkv_p[:, D:3 * D])), 5)
        put(kv, k_s, HALO, T)
        put(kv, v_s, HALO, T, D)
        hl = (_gelu(gu) * pltpu.roll(gu, 64, 1))[:, 0:64].astype(bf16)
        g = sch.add(_dot_nt(xn, _upk(wg_p[...])), 5)
        u = sch.add(_dot_nt(xn, _upk(wu_p[...])), 5)
        h = (_gelu(g) * u).astype(bf16)
        y = _dot(h, _upk(wd_p[0:FM // 2, :]))
        y = y + _dot(hl, _upk(wd_p[FM // 2:F // 2, :]))
        trig = [sch.pick(ATT_T0 + c * ATT_DT) for c in range(T // RC - len(DTRIG))]
        for n, fr in DTRIG:
            ro = min(8 * int(fr * T / 8), T - RC)
            trig.append(y[ro:ro + RC, n * 128:(n + 1) * 128])
        lnt = [sch.pick(LN_T0 + c * LN_DT) for c in range(T // RC)]
        xn_parts = []
        _attention(q_s, k_s, v_s, a_s, trig, T, False, make_ln_chunk(r_next, xn_parts, lnt))
        y = y + _dot(_upk(a_s[0:T // 2, :]), _upk(wo_p[...]))
        write_out(r_cur, T, y, True)
        xn_s[0:T // 2, :] = jnp.concatenate(xn_parts, axis=0)
        k_s[:, 0:HALO, :] = k_s[:, T:T + HALO, :]
        v_s[:, 0:HALO, :] = v_s[:, T:T + HALO, :]

    def tiles():
        def it(i, carry):
            body(i)
            return carry
        lax.fori_loop(0, NL, it, 0)

    def phase(i, carry):
        pl.when(i == 0)(prologue)
        pl.when(i == 1)(tiles)
        return carry

    lax.fori_loop(0, 2, phase, 0)
    cp(o_v, o_hbm, 0).wait()


@jax.jit
def pallas_parallel_sum__sliding_local_dilated__geglu_ffn__prompt_kernel(
    A_x: jax.Array,
    A_wqkv: jax.Array,
    A_wo: jax.Array,
    B_x: jax.Array,
    B_w_gate: jax.Array,
    B_w_up: jax.Array,
    B_w_down: jax.Array,
):
    del B_x
    anyspec = pl.BlockSpec(memory_space=pl.ANY)
    out = pl.pallas_call(
        _kernel,
        in_specs=[anyspec] * 6,
        out_specs=anyspec,
        out_shape=jax.ShapeDtypeStruct((S, D), bf16),
        scratch_shapes=[pltpu.VMEM((S, D), bf16),
                        pltpu.VMEM((S, D), bf16),
                        pltpu.VMEM((D, 3 * D), bf16),
                        pltpu.VMEM((D, D), bf16),
                        pltpu.VMEM((FM, D), bf16),
                        pltpu.VMEM((FM, D), bf16),
                        pltpu.VMEM((128, D), bf16),
                        pltpu.VMEM((F, D), bf16),
                        pltpu.VMEM((D // 2, 3 * D), u32),
                        pltpu.VMEM((D // 2, D), u32),
                        pltpu.VMEM((FM // 2, D), u32),
                        pltpu.VMEM((FM // 2, D), u32),
                        pltpu.VMEM((64, D), u32),
                        pltpu.VMEM((F // 2, D), u32),
                        pltpu.VMEM((NC, D, 128), f32),
                        pltpu.VMEM((T0, D), f32),
                        pltpu.VMEM((T0, 128), f32),
                        pltpu.VMEM((T0 // 2, D), u32),
                        pltpu.VMEM((NC, T0, 128), f32),
                        pltpu.VMEM((NC, T0 + HALO, 128), f32),
                        pltpu.VMEM((NC, T0 + HALO, 128), f32),
                        pltpu.VMEM((T0 // 2, D), u32),
                        pltpu.SemaphoreType.DMA((len(XPIECES) + 6,)),
                        pltpu.SemaphoreType.REGULAR],
        compiler_params=pltpu.CompilerParams(vmem_limit_bytes=100 * 1024 * 1024,
                                             disable_bounds_checks=True,
                                             disable_semaphore_checks=True),
    )(A_x.reshape(S, D), A_wqkv, A_wo, B_w_gate.T, B_w_up.T, B_w_down)
    return out.reshape(1, S, D)
```

```python
import jax
import jax.numpy as jnp
from jax import lax
import jax.experimental.pallas as pl
import jax.experimental.pallas.tpu as pltpu

S, D, F = 2048, 640, 1728
H, DH, W, DIL = 32, 20, 8, 2
T0 = 512
T = 384
NL = (S - T0) // T
assert T0 + NL * T == S and T <= T0
XPIECES = ((0, 128), (128, 240), (240, 352), (352, 512))
F1, F2, F3, F4 = 128, 256, 512, 1024
HALO = 16
NC = D // 128
RC = 16
FM = 1664
LOG2E = 1.4426950408889634
NT_DIMS = (((1,), (1,)), ((), ()))
ATT_T0 = 19.9
ATT_DT = 1.073
LN_T0 = 9.0
LN_DT = 0.48
DTRIG = ((0, 0), (0, 1), (1, 0), (1, 1), (2, 0), (2, 1), (3, 0), (3, 1))
P_T0 = 0.2
P_DT = 0.709
P_N = 12
P_T1 = 14.5
P_DT1 = 0.5
PLN_T0 = 0.3
PLN_DT = 0.5
PLN_OFF = 8
assert PLN_OFF + T // RC <= T0 // RC
WO_NB = 10
WO_T0 = 3.0
WO_DT = 0.286
OPIECES = (2, 3, 4)
f32 = jnp.float32
bf16 = jnp.bfloat16
u32 = jnp.uint32


def _pk(x):
    return pltpu.bitcast(x, u32)


def _upk(x):
    return pltpu.bitcast(x, bf16)


def _dot(a, b):
    return jnp.dot(a, b, preferred_element_type=f32)


def _dot_nt(a, b):
    return lax.dot_general(a, b, NT_DIMS, preferred_element_type=f32)


def _zero(v):
    return jnp.minimum(jnp.abs(v), 0.0)


def _gelu(x):
    c = 0.7978845608028654
    inner = x * (c + (c * 0.044715) * (x * x))
    return (0.5 * x) * (1.0 + jnp.tanh(inner))


def _ln(x, z=None):
    x = x.astype(f32)
    t = x[:, 0:128] if z is None else z + x[:, 0:128]
    for j in range(1, NC):
        t = t + x[:, j * 128:(j + 1) * 128]
    m = jnp.sum(t, axis=-1, keepdims=True) * (1.0 / D)
    xc = x - m
    var = jnp.mean(xc * xc, axis=-1, keepdims=True)
    rstd = lax.rsqrt(var + 1e-5)
    return (xc * rstd).astype(bf16), rstd


def _perm_cols(src_ref, dst_ref, p):
    R = D // 2
    lane = lax.broadcasted_iota(jnp.int32, (8, 128), 1)
    outs = []
    for j in range(NC):
        rel = (lane + (128 - 4 * j)) & 127
        h = (13 * (rel >> 2)) & 31
        c = jnp.tile(20 * h + 4 * j + (rel & 3), (R // 8, 1))
        idx = jnp.tile((20 * (lane & 31) + 4 * j + (lane >> 5)) & 127, (R // 8, 1))
        w = [_pk(src_ref[:, p * D + i * 128: p * D + (i + 1) * 128]) for i in range(NC)]
        s = w[4]
        for i in (3, 2, 1, 0):
            s = jnp.where(c < 128 * (i + 1), w[i], s)
        g = jnp.take_along_axis(s, idx, axis=1)
        dst_ref[:, p * D + j * 128: p * D + (j + 1) * 128] = g
        outs.append(_upk(g))
    return jnp.concatenate(outs, axis=1)


def _perm_rows(tmp_ref, dst_ref):
    cols = []
    for j in range(NC):
        blk = jnp.concatenate(
            [tmp_ref[j, pl.ds(d, H, stride=DH), :].astype(bf16) for d in range(DH)], axis=0)
        dst_ref[:, j * 128:(j + 1) * 128] = _pk(blk)
        cols.append(blk)
    return jnp.concatenate(cols, axis=1)


class _Sched:
    def __init__(self, rows, first_pass):
        self.rows, self.p, self.tiles = rows, first_pass, []

    def add(self, val, k_tiles):
        for n in range(val.shape[1] // 128):
            self.p += k_tiles
            self.tiles.append(((self.p - 1) // 4, val[:, n * 128:(n + 1) * 128]))
        return val

    def pick(self, t):
        for rnd, val in self.tiles:
            if rnd + 1 <= t:
                continue
            ro = min(8 * int(max(t - rnd, 0.0) * self.rows / 8), self.rows - RC)
            return val[ro:ro + RC]
        return self.tiles[-1][1][self.rows - RC:self.rows]


def _attention(q_s, k_s, v_s, a_s, trig, rows, first, ln_chunk):
    qs = (DH ** -0.5) * LOG2E
    for c in range(rows // RC):
        r0 = c * RC
        sc = qs + _zero(trig[c])
        rstd = ln_chunk(c)
        if rstd is not None:
            sc = sc + jnp.minimum(rstd, 0.0)
        q = [q_s[j, r0:r0 + RC, :] * sc for j in range(NC)]
        ls = []
        for w in range(W):
            off = HALO + r0 - DIL * w
            p = q[0] * k_s[0, off:off + RC, :]
            for j in range(1, NC):
                p = p + q[j] * k_s[j, off:off + RC, :]
            p = p + pltpu.roll(p, 64, 1)
            p = p + pltpu.roll(p, 32, 1)
            if first and r0 < DIL * w:
                rows_i = r0 + lax.broadcasted_iota(jnp.int32, (RC, 128), 0)
                p = jnp.where(rows_i >= DIL * w, p, -1e9 * LOG2E)
            ls.append(p)
        mx = jnp.maximum(jnp.maximum(jnp.maximum(ls[0], ls[1]), jnp.maximum(ls[2], ls[3])),
                         jnp.maximum(jnp.maximum(ls[4], ls[5]), jnp.maximum(ls[6], ls[7])))
        es = [jnp.exp2(l - mx) for l in ls]
        den = ((es[0] + es[1]) + (es[2] + es[3])) + ((es[4] + es[5]) + (es[6] + es[7]))
        inv = pl.reciprocal(den, approx=True)
        inv = inv * (2.0 - den * inv)
        for j in range(NC):
            acc = None
            for w in range(W):
                off = HALO + r0 - DIL * w
                t = es[w] * v_s[j, off:off + RC, :]
                acc = t if acc is None else acc + t
            a_s[r0 // 2:(r0 + RC) // 2, j * 128:(j + 1) * 128] = _pk((acc * inv).astype(bf16))


def _kernel(x_hbm, wqkv_hbm, wo_hbm, wg_hbm, wu_hbm, wd_hbm, o_hbm,
            x_v, o_v, wqkv_raw, wo_raw, wg_v, wu_v, wl_v, wd_v,
            wqkv_p, wo_p, wg_p, wu_p, wl_p, wd_p, wo_tmp, h_s, y_s,
            xn_s, q_s, k_s, v_s, a_s, sem, sem_b):
    NXP = len(XPIECES)

    def cp(src, dst, s):
        return pltpu.make_async_copy(src, dst, sem.at[s])

    def fence():
        pl.semaphore_signal(sem_b, 1)
        pl.semaphore_wait(sem_b, 1)

    def rows_cp(src, dst, a, b, s):
        return cp(src.at[a:b], dst.at[a:b], s)

    xp_cp = [rows_cp(x_hbm, x_v, a, b, p) for p, (a, b) in enumerate(XPIECES)]

    def pair_cp(a, b, s):
        return [rows_cp(wg_hbm, wg_v, a, b, s), rows_cp(wu_hbm, wu_v, a, b, s)]

    g1 = pair_cp(0, F1, NXP)
    g2 = pair_cp(F1, F2, NXP + 1)
    g3 = pair_cp(F2, F3, NXP + 2) + [rows_cp(wd_hbm, wd_v, 0, 128, NXP + 2)]
    g4 = pair_cp(F3, F4, NXP + 3) + [rows_cp(wd_hbm, wd_v, 128, 256, NXP + 3),
                                     cp(wg_hbm.at[FM:F], wl_v.at[0:64], NXP + 3),
                                     cp(wu_hbm.at[FM:F], wl_v.at[64:128], NXP + 3)]
    g5 = [rows_cp(wd_hbm, wd_v, 256, 384, NXP + 4),
          cp(wqkv_hbm, wqkv_raw, NXP + 4), cp(wo_hbm, wo_raw, NXP + 4)]
    g6 = pair_cp(F4, FM, NXP + 5) + [rows_cp(wd_hbm, wd_v, 384, F, NXP + 5),
                                     rows_cp(x_hbm, x_v, T0, T0 + T, NXP + 5)]
    xr_cp = rows_cp(x_hbm, x_v, T0 + T, S, 1)

    for g in [[c] for c in xp_cp[:-1]] + [g1, xp_cp[-1:], g2, g3, g4, g5, g6]:
        for c in g:
            c.start()
        fence()

    k_s[:, 0:HALO, :] = jnp.zeros((NC, HALO, 128), f32)
    v_s[:, 0:HALO, :] = jnp.zeros((NC, HALO, 128), f32)

    def gate(xn, a, b):
        wg = wg_v[a:b, :]
        wg_p[a // 2:b // 2, :] = _pk(wg)
        return _dot_nt(xn, wg)

    def up(xn, a, b):
        wu = wu_v[a:b, :]
        wu_p[a // 2:b // 2, :] = _pk(wu)
        return _dot_nt(xn, wu)

    def act(g, u):
        return _pk((_gelu(g) * u).astype(bf16))

    def put(r, dst, off, rows, c0=0):
        for j in range(NC):
            dst[j, off:off + rows, :] = r[:, c0 + j * 128:c0 + (j + 1) * 128]

    def make_ln_chunk(r_next, outs, trig, off=0):
        def ln_chunk(c):
            c = c - off
            if c < 0 or c * RC >= T:
                return None
            if isinstance(r_next, int):
                xx = x_v[r_next + c * RC:r_next + (c + 1) * RC, :]
            else:
                xx = x_v[pl.ds(pl.multiple_of(r_next + c * RC, 16), RC), :]
            y, rstd = _ln(xx, _zero(trig[c]))
            outs.append(_pk(y))
            return rstd
        return ln_chunk

    def write_out(r, rows, y, split):
        if not split:
            o_v[pl.ds(r, rows), :] = (x_v[pl.ds(r, rows), :].astype(f32) + y).astype(bf16)
            cp(o_v.at[pl.ds(r, rows)], o_hbm.at[pl.ds(r, rows)], 0).start()
            return
        lo = 0
        for j in range(NC):
            cs = slice(j * 128, (j + 1) * 128)
            o_v[pl.ds(r, rows), cs] = (x_v[pl.ds(r, rows), cs].astype(f32) + y[:, cs]).astype(bf16)
            if j in OPIECES:
                ps = slice(lo, (j + 1) * 128)
                lo = (j + 1) * 128
                cp(o_v.at[pl.ds(r, rows), ps], o_hbm.at[pl.ds(r, rows), ps], 0).start()

    RA = XPIECES[-1][0]

    def ffn(xn, a, b, r0, r1):
        h_s[r0 // 2:r1 // 2, a:b] = act(gate(xn, a, b), up(xn, a, b))

    def last_tile(xn):
        wl = wl_v[...]
        wl_p[...] = _pk(wl)
        gu = _dot_nt(xn, wl)
        h_s[:, F4:F4 + 128] = act(gu, pltpu.roll(gu, 64, 1))

    def region1():
        for (a, b), c in list(zip(XPIECES, xp_cp))[:-1]:
            c.wait()
            xn_s[a // 2:b // 2, :] = _pk(_ln(x_v[a:b, :])[0])
        for c in g1:
            c.wait()
        ffn(_upk(xn_s[0:RA // 2, :]), 0, F1, 0, RA)

    def region2():
        for c in xp_cp[-1:] + g2:
            c.wait()
        xb = _pk(_ln(x_v[RA:T0, :])[0])
        xn_s[RA // 2:T0 // 2, :] = xb
        ffn(_upk(xn_s[0:RA // 2, :]), F1, F2, 0, RA)
        xb = _upk(xb)
        h_s[RA // 2:T0 // 2, 0:F2] = act(_dot_nt(xb, wg_v[0:F2, :]), _dot_nt(xb, wu_v[0:F2, :]))

    def down(h, a, b):
        wd = wd_v[a:b, :]
        wd_p[a // 2:b // 2, :] = _pk(wd)
        return _dot(h, wd)

    def region3():
        for c in g3:
            c.wait()
        y_s[...] = down(_upk(h_s[:, 0:128]), 0, 128)
        ffn(_upk(xn_s[...]), F2, F3, 0, T0)

    def region45():
        for c in g4:
            c.wait()
        xn = _upk(xn_s[...])
        y_s[...] = y_s[...] + down(_upk(h_s[:, 128:256]), 128, 256)
        last_tile(xn)
        ffn(xn, F3, F4, 0, T0)
        for c in g5:
            c.wait()
        wq = _perm_cols(wqkv_raw, wqkv_p, 0)
        wk = _perm_cols(wqkv_raw, wqkv_p, 1)
        wv = _perm_cols(wqkv_raw, wqkv_p, 2)
        sch = _Sched(T0, 0)
        y_s[...] = sch.add(y_s[...] + down(_upk(h_s[:, 256:384]), 256, 384), 1)
        put(sch.add(_dot(xn, wq), 5), q_s, 0, T0)
        put(sch.add(_dot(xn, wk), 5), k_s, HALO, T0)
        put(sch.add(_dot(xn, wv), 5), v_s, HALO, T0)
        rb = D // WO_NB
        for j in range(NC):
            for b in range(WO_NB):
                z = jnp.tile(_zero(sch.pick(WO_T0 + (j * WO_NB + b) * WO_DT)), (rb // RC, 1))
                wo_tmp[j, b * rb:(b + 1) * rb, :] = (
                    wo_raw[b * rb:(b + 1) * rb, j * 128:(j + 1) * 128].astype(f32) + z)

    def region6():
        for c in g6:
            c.wait()
        xr_cp.start()
        xn = _upk(xn_s[...])
        sch = _Sched(T0, -2)
        wd0 = jnp.concatenate([wd_v[384:512, :], wd_v[FM:F, :]], axis=0)
        wd_p[192:256, :] = _pk(wd0[0:128])
        wd_p[FM // 2:F // 2, :] = _pk(wd0[128:192])
        hx = jnp.concatenate([_upk(h_s[:, 384:512]), _upk(h_s[:, F4:F4 + 128])[:, 0:64]], axis=1)
        y = sch.add(y_s[...] + _dot(hx, wd0), 2)
        gb = sch.add(gate(xn, F4, FM), 5)
        ub = sch.add(up(xn, F4, FM), 5)
        hp = jnp.concatenate([h_s[:, 512:F4], act(gb, ub)], axis=1)
        for lo, hi in ((512, 768), (768, 1280), (1280, FM)):
            y = sch.add(y + down(_upk(hp[:, lo - 512:hi - 512]), lo, hi), (hi - lo) // 128)
        trig = [sch.pick(P_T0 + c * P_DT) for c in range(P_N)]
        trig += [sch.pick(P_T1 + c * P_DT1) for c in range(T0 // RC - P_N)]
        lnt = [sch.pick(PLN_T0 + c * PLN_DT) for c in range(T // RC)]
        xn_parts = []
        _attention(q_s, k_s, v_s, a_s, trig, T0, True, make_ln_chunk(T0, xn_parts, lnt, PLN_OFF))
        wo = _perm_rows(wo_tmp, wo_p)
        y = y + _dot(_upk(a_s[0:T0 // 2, :]), wo)
        write_out(0, T0, y, False)
        xn_s[0:T // 2, :] = jnp.concatenate(xn_parts, axis=0)
        k_s[:, 0:HALO, :] = k_s[:, T0:T0 + HALO, :]
        v_s[:, 0:HALO, :] = v_s[:, T0:T0 + HALO, :]
        xr_cp.wait()

    def body(i):
        r_cur = pl.multiple_of(T0 + i * T, 16)
        inext = jnp.minimum(i + 1, NL - 1)
        r_next = pl.multiple_of(T0 + inext * T, 16)
        xn = _upk(xn_s[0:T // 2, :])
        sch = _Sched(T, -1)
        put(sch.add(_dot(xn, _upk(wqkv_p[:, 0:D])), 5), q_s, 0, T)
        gu = sch.add(_dot_nt(xn, _upk(wl_p[...])), 5)
        kv = sch.add(_dot(xn, _upk(wqkv_p[:, D:3 * D])), 5)
        put(kv, k_s, HALO, T)
        put(kv, v_s, HALO, T, D)
        hl = (_gelu(gu) * pltpu.roll(gu, 64, 1))[:, 0:64].astype(bf16)
        g = sch.add(_dot_nt(xn, _upk(wg_p[...])), 5)
        u = sch.add(_dot_nt(xn, _upk(wu_p[...])), 5)
        h = (_gelu(g) * u).astype(bf16)
        y = _dot(h, _upk(wd_p[0:FM // 2, :]))
        y = y + _dot(hl, _upk(wd_p[FM // 2:F // 2, :]))
        trig = [sch.pick(ATT_T0 + c * ATT_DT) for c in range(T // RC - len(DTRIG))]
        for n, fr in DTRIG:
            ro = min(8 * int(fr * T / 8), T - RC)
            trig.append(y[ro:ro + RC, n * 128:(n + 1) * 128])
        lnt = [sch.pick(LN_T0 + c * LN_DT) for c in range(T // RC)]
        xn_parts = []
        _attention(q_s, k_s, v_s, a_s, trig, T, False, make_ln_chunk(r_next, xn_parts, lnt))
        y = y + _dot(_upk(a_s[0:T // 2, :]), _upk(wo_p[...]))
        write_out(r_cur, T, y, True)
        xn_s[0:T // 2, :] = jnp.concatenate(xn_parts, axis=0)
        k_s[:, 0:HALO, :] = k_s[:, T:T + HALO, :]
        v_s[:, 0:HALO, :] = v_s[:, T:T + HALO, :]

    def tiles():
        def it(i, carry):
            body(i)
            return carry
        lax.fori_loop(0, NL, it, 0)

    def phase(i, carry):
        pl.when(i == 0)(region1)
        pl.when(i <= 0)(region2)
        pl.when(i < 1)(region3)
        pl.when(i != 1)(region45)
        pl.when(i == 1)(region6)
        pl.when(i >= 1)(tiles)
        return carry

    lax.fori_loop(0, 2, phase, 0)
    cp(o_v, o_hbm, 0).wait()


@jax.jit
def pallas_parallel_sum__sliding_local_dilated__geglu_ffn__prompt_kernel(
    A_x: jax.Array,
    A_wqkv: jax.Array,
    A_wo: jax.Array,
    B_x: jax.Array,
    B_w_gate: jax.Array,
    B_w_up: jax.Array,
    B_w_down: jax.Array,
):
    del B_x
    anyspec = pl.BlockSpec(memory_space=pl.ANY)
    out = pl.pallas_call(
        _kernel,
        in_specs=[anyspec] * 6,
        out_specs=anyspec,
        out_shape=jax.ShapeDtypeStruct((S, D), bf16),
        scratch_shapes=[pltpu.VMEM((S, D), bf16),
                        pltpu.VMEM((S, D), bf16),
                        pltpu.VMEM((D, 3 * D), bf16),
                        pltpu.VMEM((D, D), bf16),
                        pltpu.VMEM((FM, D), bf16),
                        pltpu.VMEM((FM, D), bf16),
                        pltpu.VMEM((128, D), bf16),
                        pltpu.VMEM((F, D), bf16),
                        pltpu.VMEM((D // 2, 3 * D), u32),
                        pltpu.VMEM((D // 2, D), u32),
                        pltpu.VMEM((FM // 2, D), u32),
                        pltpu.VMEM((FM // 2, D), u32),
                        pltpu.VMEM((64, D), u32),
                        pltpu.VMEM((F // 2, D), u32),
                        pltpu.VMEM((NC, D, 128), f32),
                        pltpu.VMEM((T0 // 2, F4 + 128), u32),
                        pltpu.VMEM((T0, D), f32),
                        pltpu.VMEM((T0 // 2, D), u32),
                        pltpu.VMEM((NC, T0, 128), f32),
                        pltpu.VMEM((NC, T0 + HALO, 128), f32),
                        pltpu.VMEM((NC, T0 + HALO, 128), f32),
                        pltpu.VMEM((T0 // 2, D), u32),
                        pltpu.SemaphoreType.DMA((len(XPIECES) + 6,)),
                        pltpu.SemaphoreType.REGULAR],
        compiler_params=pltpu.CompilerParams(vmem_limit_bytes=100 * 1024 * 1024,
                                             disable_bounds_checks=True,
                                             disable_semaphore_checks=True),
    )(A_x.reshape(S, D), A_wqkv, A_wo, B_w_gate.T, B_w_up.T, B_w_down)
    return out.reshape(1, S, D)
```
